```python
import jax
import jax.numpy as jnp

def _softmax(x, axis=-1):
    return jax.nn.softmax(x, axis=axis)

def _gelu(x):
    return jax.nn.gelu(x, approximate=True)

def _silu(x):
    return jax.nn.silu(x)

def _sigmoid(x):
    return jax.nn.sigmoid(x)

def _layernorm(x, axis=-1, eps=1e-05):
    m = jnp.mean(x, axis=axis, keepdims=True)
    v = jnp.var(x, axis=axis, keepdims=True)
    return (x - m) / jnp.sqrt(v + eps)

def _scatter_add(tgt, idx, src, axis=0):
    return tgt.at[idx].add(src)

def _segment_sum(src, seg, n):
    return jax.ops.segment_sum(src, seg, n)

class _Rng:

    def __init__(self, key):
        self._k = key

    def _next(self):
        self._k, sub = jax.random.split(self._k)
        return sub

    def normal(self, shape):
        return jax.random.normal(self._next(), shape, dtype=jnp.bfloat16)

    def randint(self, lo, hi, shape):
        return jax.random.randint(self._next(), shape, lo, hi, dtype=jnp.int32)

    def uniform(self, shape, lo=0.0, hi=1.0):
        return jax.random.uniform(self._next(), shape, jnp.bfloat16, lo, hi)

    def permutation(self, n):
        return jax.random.permutation(self._next(), n)
kernel_name = 'adaLN_cond__sliding_block_cached__mixer_token_mlp__decode'

def setup_inputs():
    _rng = _Rng(jax.random.key(int.from_bytes(__import__("os").urandom(4), "little")))
    _w = lambda a: (lambda t: t.astype(jnp.bfloat16) if jnp.issubdtype(t.dtype, jnp.floating) else t)(jnp.asarray(a))

    def _A_setup():
        B, Sq, D = (1, 1, 640)
        Hq, Hkv, Sk, Dh = (32, 32, 32768, 192)
        assert Hq % Hkv == 0, (Hq, Hkv)
        return {'x': _w((lambda *s: _rng.normal(s) * 0.05)(B, Sq, D)), 'k_cache': _w((lambda *s: _rng.normal(s) * 0.05)(B, Hkv, Sk, Dh)), 'v_cache': _w((lambda *s: _rng.normal(s) * 0.05)(B, Hkv, Sk, Dh)), 'wq': _w((lambda *s: _rng.normal(s) * 0.05)(D, Hq * Dh) * D ** (-0.5)), 'wo': _w((lambda *s: _rng.normal(s) * 0.05)(Hq * Dh, D) * (Hq * Dh) ** (-0.5))}
    _A_in = _A_setup()

    def _B_setup():
        B, S, D, F = (1, 1, 640, 1536)
        return {'x': _w((lambda *s: _rng.normal(s) * 0.05)(B, S, D)), 'w1': _w((lambda *s: _rng.normal(s) * 0.05)(S, F) * S ** (-0.5)), 'b1': _w((lambda *s: _rng.normal(s) * 0.05)(F) * 0.02), 'w2': _w((lambda *s: _rng.normal(s) * 0.05)(F, S) * F ** (-0.5)), 'b2': _w((lambda *s: _rng.normal(s) * 0.05)(S) * 0.02)}
    _B_in = _B_setup()
    return {'A_x': _A_in['x'], 'A_k_cache': _A_in['k_cache'], 'A_v_cache': _A_in['v_cache'], 'A_wq': _A_in['wq'], 'A_wo': _A_in['wo'], 'B_x': _B_in['x'], 'B_w1': _B_in['w1'], 'B_b1': _B_in['b1'], 'B_w2': _B_in['w2'], 'B_b2': _B_in['b2'], 'c': _w((lambda *s: _rng.normal(s) * 0.05)(1, 640)), 'w_mod': _w((lambda *s: _rng.normal(s) * 0.05)(640, 6 * 640) * 640 ** (-0.5))}

def reference(A_x, A_k_cache, A_v_cache, A_wq, A_wo, B_x, B_w1, B_b1, B_w2, B_b2, c, w_mod):

    def _A_ref(x, k_cache, v_cache, wq, wo):
        B, Sq, D = x.shape
        Hq, Dh = (32, 192)
        Hkv, Sk = (k_cache.shape[1], k_cache.shape[2])
        W = min(4096, max(256, Sk // 4))
        rep = Hq // Hkv
        q = (lambda x, *d: x.transpose(*d))((x @ wq).reshape(B, Sq, Hq, Dh), 0, 2, 1, 3)
        k = jnp.repeat(k_cache[:, :, Sk - W:, :], rep, axis=1)
        v = jnp.repeat(v_cache[:, :, Sk - W:, :], rep, axis=1)
        scores = jnp.einsum('bhqd,bhkd->bhqk', q, k) * Dh ** (-0.5)
        p = _softmax(scores, axis=-1)
        o = jnp.einsum('bhqk,bhkd->bhqd', p, v)
        return (lambda x, *d: x.transpose(*d))(o, 0, 2, 1, 3).reshape(B, Sq, Hq * Dh) @ wo

    def _B_ref(x, w1, b1, w2, b2):
        B, S, D = x.shape
        h = _layernorm(x, axis=-1)
        u = jnp.einsum('bsd,sf->bdf', h, w1) + b1
        u = _gelu(u)
        y = jnp.einsum('bdf,fs->bds', u, w2) + b2
        return (lambda x, *d: x.transpose(*d))(y, 0, 2, 1)
    x = A_x
    mod = (_silu(c) @ w_mod).reshape(c.shape[0], 6, 1, -1)
    sa, ca, ga, sb, cb, gb = (mod[:, 0].copy(), mod[:, 1].copy(), mod[:, 2].copy(), mod[:, 3].copy(), mod[:, 4].copy(), mod[:, 5].copy())
    h = _layernorm(x, axis=-1) * (1 + ca) + sa
    x = x + ga * _A_ref(h, A_k_cache, A_v_cache, A_wq, A_wo)
    h = _layernorm(x, axis=-1) * (1 + cb) + sb
    x = x + gb * _B_ref(h, B_w1, B_b1, B_w2, B_b2)
    return x
```

```python
import jax
import jax.numpy as jnp
import numpy as np
from jax import lax
import jax.experimental.pallas as pl
import jax.experimental.pallas.tpu as pltpu

D = 640
HQ = 32
DH = 192
SK = 32768
W = 4096
F = 1536
f32 = jnp.float32
bf16 = jnp.bfloat16
C0 = float(np.sqrt(2.0 / np.pi))
C1 = 0.044715 * C0


def _ln(x):
    m = jnp.mean(x, axis=-1, keepdims=True)
    xc = x - m
    v = jnp.mean(xc * xc, axis=-1, keepdims=True)
    return xc / jnp.sqrt(v + 1e-5)


NBUF = 4
CH = 32
PRIO = 0
GB_AT = 1
UNROLL = True


def _kernel(x_hbm, k_hbm, v_hbm, wq_hbm, wo_hbm, w1_hbm, b1_hbm, w2_hbm, b2_hbm, c_hbm, wm_hbm,
          o_ref,
          kbuf, vbuf, wq_v, wo_v, wm_v, x_v, w1_v, b1_v, w2_v, b2_v, c_v, q_s, w1b, b1b, w2b,
          ksem, vsem, wsem, msem, ssem):
  def kcopy(h, slot):
      return pltpu.make_async_copy(k_hbm.at[0, h, :, pl.ds(SK - W, W)], kbuf.at[slot], ksem.at[slot])

  def vcopy(h, slot):
      return pltpu.make_async_copy(v_hbm.at[0, h, :, pl.ds(SK - W, W)], vbuf.at[slot], vsem.at[slot])

  small = [pltpu.make_async_copy(s, d, ssem.at[i]) for i, (s, d) in enumerate(
      [(c_hbm, c_v), (x_hbm, x_v), (w1_hbm, w1_v), (b1_hbm, b1_v), (w2_hbm, w2_v), (b2_hbm, b2_v)])]
  mcp = [pltpu.make_async_copy(wm_hbm.at[:, pl.ds(i * D, D)], wm_v.at[i], msem.at[i]) for i in range(6)]
  wq_cp = pltpu.make_async_copy(wq_hbm, wq_v, wsem.at[0])
  wo_cp = pltpu.make_async_copy(wo_hbm, wo_v, wsem.at[1])
  mcp[0].start()
  mcp[1].start(priority=PRIO)
  for s in small:
      s.start()
  wq_cp.start()
  kcopy(0, 0).start(priority=PRIO)
  vcopy(0, 0).start(priority=PRIO)
  wo_cp.start()
  for i in range(1, NBUF):
      kcopy(i, i).start()
      vcopy(i, i).start(priority=PRIO)
  for s in small:
      s.wait()
  c = c_v[...].astype(f32)
  sc = (c * jax.nn.sigmoid(c)).astype(bf16)
  x = x_v[0].astype(f32)
  xn = _ln(x)
  w1 = w1_v[...].astype(f32)
  b1 = b1_v[...].astype(f32).reshape(1, F)
  hw2 = 0.5 * w2_v[...].astype(f32)
  b2 = b2_v[...].astype(f32).reshape(1, 1)
  w1b[...] = jnp.broadcast_to(w1, (128, F)).T
  b1b[...] = jnp.broadcast_to(b1, (128, F)).T
  w2b[...] = jnp.broadcast_to(hw2, (128, F)).T
  lin1 = jnp.sum(hw2 * w1, axis=-1, keepdims=True)
  lin0 = jnp.sum(hw2 * b1, axis=-1, keepdims=True) + b2

  def mod(i):
      mcp[i].wait()
      return jnp.dot(sc, wm_v[i], preferred_element_type=f32)

  sa = mod(0)
  ca = mod(1)
  h = xn * (1 + ca) + sa
  wq_cp.wait()
  q = jnp.dot(h.astype(bf16), wq_v[...], preferred_element_type=f32) * (DH ** -0.5)
  for i in range(HQ):
      q_s[i:i + 1, :] = q[:, i * DH:(i + 1) * DH]
  wo_cp.wait()

  def body(hd, acc):
      slot = hd % NBUF
      kcopy(hd, slot).wait()
      qh = q_s[pl.ds(hd, 1), :].astype(bf16)
      s = jnp.dot(qh, kbuf[slot], preferred_element_type=f32)

      @pl.when(hd + NBUF < HQ)
      def _():
          kcopy(hd + NBUF, slot).start()
      for j in range(3):
          @pl.when(hd + NBUF == HQ + j)
          def _():
              mcp[2 + j].start()
      m = jnp.max(s, axis=-1, keepdims=True)
      p = jnp.exp(s - m)
      l = jnp.sum(p, axis=-1, keepdims=True)
      vcopy(hd, slot).wait()
      o = lax.dot_general(p.astype(bf16), vbuf[slot], (((1,), (1,)), ((), ())), preferred_element_type=f32)

      @pl.when(hd + NBUF < HQ)
      def _():
          vcopy(hd + NBUF, slot).start(priority=PRIO)
      o = o / l
      woh = wo_v[pl.ds(pl.multiple_of(hd * DH, DH), DH), :]
      return acc + jnp.dot(o.astype(bf16), woh, preferred_element_type=f32)

  a = lax.fori_loop(0, HQ, body, jnp.zeros((1, D), f32))
  if GB_AT == 0:
      mcp[5].start()
  ga = mod(2)
  if GB_AT == 1:
      mcp[5].start()
  x1 = x + ga * a
  x1n = _ln(x1)
  sb = mod(3)
  if GB_AT == 2:
      mcp[5].start()
  cb = mod(4)
  if GB_AT == 3:
      mcp[5].start()
  h3 = _ln(x1n * (1 + cb) + sb)
  hs = [jnp.broadcast_to(h3[:, j * 128:(j + 1) * 128], (CH, 128)) for j in range(D // 128)]

  def mlp(i, accs):
      r = pl.ds(pl.multiple_of(i * CH, CH), CH)
      w1c, b1c, w2c = w1b[r, :], b1b[r, :], w2b[r, :]
      out = []
      for j in range(D // 128):
          u = w1c * hs[j] + b1c
          t = jnp.tanh(u * (C0 + C1 * (u * u)))
          g = (u * w2c) * t
          out.append(accs[j] + g.reshape(CH // 8, 8, 128).sum(axis=0))
      return tuple(out)

  accs = lax.fori_loop(0, F // CH, mlp, tuple(jnp.zeros((8, 128), f32) for _ in range(D // 128)), unroll=UNROLL)
  y = jnp.concatenate([jnp.sum(t, axis=0, keepdims=True) for t in accs], axis=-1) + (lin1 * h3 + lin0)
  gb = mod(5)
  o_ref[0] = (x1 + gb * y).astype(o_ref.dtype)

@jax.jit
def pallas_adaLN_cond__sliding_block_cached__mixer_token_mlp__decode_kernel(A_x, A_k_cache, A_v_cache, A_wq, A_wo, B_x, B_w1, B_b1, B_w2, B_b2, c, w_mod):
  kT = jnp.swapaxes(A_k_cache, 2, 3)
  vT = jnp.swapaxes(A_v_cache, 2, 3)
  w2 = B_w2.reshape(1, F)
  return pl.pallas_call(
      _kernel,
      in_specs=[pl.BlockSpec(memory_space=pl.ANY)] * 11,
      out_specs=pl.BlockSpec(memory_space=pltpu.VMEM),
      out_shape=jax.ShapeDtypeStruct((1, 1, D), A_x.dtype),
      scratch_shapes=[
          pltpu.VMEM((NBUF, DH, W), bf16), pltpu.VMEM((NBUF, DH, W), bf16),
          pltpu.VMEM((D, HQ * DH), bf16), pltpu.VMEM((HQ * DH, D), bf16), pltpu.VMEM((6, D, D), bf16),
          pltpu.VMEM((1, 1, D), bf16), pltpu.VMEM((1, F), bf16), pltpu.VMEM((F,), bf16),
          pltpu.VMEM((1, F), bf16), pltpu.VMEM((1,), bf16), pltpu.VMEM((1, D), bf16),
          pltpu.VMEM((HQ, DH), f32),
          pltpu.VMEM((F, 128), f32), pltpu.VMEM((F, 128), f32), pltpu.VMEM((F, 128), f32),
          pltpu.SemaphoreType.DMA((NBUF,)), pltpu.SemaphoreType.DMA((NBUF,)),
          pltpu.SemaphoreType.DMA((2,)), pltpu.SemaphoreType.DMA((6,)), pltpu.SemaphoreType.DMA((6,)),
      ],
      compiler_params=pltpu.CompilerParams(vmem_limit_bytes=100 * 1024 * 1024),
  )(A_x, kT, vT, A_wq, A_wo, B_w1, B_b1, w2, B_b2, c, w_mod)
```

```python
import jax
import jax.numpy as jnp
import numpy as np
from jax import lax
import jax.experimental.pallas as pl
import jax.experimental.pallas.tpu as pltpu

D = 640
HQ = 32
DH = 192
SK = 32768
W = 4096
F = 1536
f32 = jnp.float32
bf16 = jnp.bfloat16
C0 = float(np.sqrt(2.0 / np.pi))
C1 = 0.044715 * C0
S3 = float(C1 ** (1.0 / 3.0))


def _ln(x):
    m = jnp.mean(x, axis=-1, keepdims=True)
    xc = x - m
    v = jnp.mean(xc * xc, axis=-1, keepdims=True)
    return xc / jnp.sqrt(v + 1e-5)


NBUF = 3
CH = 128
GB_AT = -1
MXU = 1
EV = (60, 61, 62, 63)


def _kernel(x_hbm, k_hbm, v_hbm, wq_hbm, wo_hbm, w1_hbm, b1_hbm, w2_hbm, b2_hbm, c_hbm, wm_hbm,
          o_ref,
          kbuf, vbuf, wq_v, wo_v, wm_v, x_v, w1_v, b1_v, w2_v, b2_v, c_v, q_s, w1b, b1b, w2b,
          ksem, vsem, wsem, msem, ssem):
  def kcopy(h, slot):
      return pltpu.make_async_copy(k_hbm.at[0, h, :, pl.ds(SK - W, W)], kbuf.at[slot], ksem.at[slot])

  def vcopy(h, slot):
      return pltpu.make_async_copy(v_hbm.at[0, h, :, pl.ds(SK - W, W)], vbuf.at[slot], vsem.at[slot])

  small = [pltpu.make_async_copy(s, d, ssem.at[i]) for i, (s, d) in enumerate(
      [(c_hbm, c_v), (x_hbm, x_v), (w1_hbm, w1_v), (b1_hbm, b1_v), (w2_hbm, w2_v), (b2_hbm, b2_v)])]
  mcp = [pltpu.make_async_copy(wm_hbm.at[:, pl.ds(i * D, D)], wm_v.at[i], msem.at[i]) for i in range(6)]
  wq_cp = pltpu.make_async_copy(wq_hbm, wq_v, wsem.at[0])
  wo_cp = pltpu.make_async_copy(wo_hbm, wo_v, wsem.at[1])
  mcp[0].start()
  mcp[1].start()
  for s in small:
      s.start()
  wq_cp.start()
  kcopy(0, 0).start()
  vcopy(0, 0).start()
  wo_cp.start()
  for i in range(1, NBUF):
      kcopy(i, i).start()
      vcopy(i, i).start()
  for s in small:
      s.wait()
  c = c_v[...].astype(f32)
  sc = (c * jax.nn.sigmoid(c)).astype(bf16)
  x = x_v[0].astype(f32)
  xn = _ln(x)
  w1 = w1_v[...].astype(f32)
  b1 = b1_v[...].astype(f32).reshape(1, F)
  hw2 = 0.5 * w2_v[...].astype(f32)
  b2 = b2_v[...].astype(f32).reshape(1, 1)
  w1b[...] = jnp.broadcast_to(w1 * S3, (128, F)).T
  b1b[...] = jnp.broadcast_to(b1 * S3, (128, F)).T
  if not MXU:
      w2b[...] = jnp.broadcast_to(hw2 * (1.0 / S3), (128, F)).T
  lin1 = jnp.sum(hw2 * w1, axis=-1, keepdims=True)
  lin0 = jnp.sum(hw2 * b1, axis=-1, keepdims=True) + b2

  def mod(i):
      mcp[i].wait()
      return jnp.dot(sc, wm_v[i], preferred_element_type=f32)

  sa = mod(0)
  ca = mod(1)
  h = xn * (1 + ca) + sa
  wq_cp.wait()
  q = jnp.dot(h.astype(bf16), wq_v[...], preferred_element_type=f32) * (DH ** -0.5)
  for i in range(HQ):
      q_s[i:i + 1, :] = q[:, i * DH:(i + 1) * DH]
  wo_cp.wait()

  def body(hd, acc):
      slot = hd % NBUF
      kcopy(hd, slot).wait()
      qh = q_s[pl.ds(hd, 1), :].astype(bf16)
      s = jnp.dot(qh, kbuf[slot], preferred_element_type=f32)

      @pl.when(hd + NBUF < HQ)
      def _():
          kcopy(hd + NBUF, slot).start()
      def late(stage):
          for j, e in enumerate(EV):
              if e % 2 == stage:
                  pl.when(hd == e // 2)(mcp[2 + j].start)
      late(0)
      m = jnp.max(s, axis=-1, keepdims=True)
      p = jnp.exp(s - m)
      l = jnp.sum(p, axis=-1, keepdims=True)
      vcopy(hd, slot).wait()
      o = lax.dot_general(p.astype(bf16), vbuf[slot], (((1,), (1,)), ((), ())), preferred_element_type=f32)

      @pl.when(hd + NBUF < HQ)
      def _():
          vcopy(hd + NBUF, slot).start()
      late(1)
      o = o / l
      woh = wo_v[pl.ds(pl.multiple_of(hd * DH, DH), DH), :]
      return acc + jnp.dot(o.astype(bf16), woh, preferred_element_type=f32)

  a = lax.fori_loop(0, HQ, body, jnp.zeros((1, D), f32))
  ga = mod(2)
  if GB_AT == 1:
      mcp[5].start()
  x1 = x + ga * a
  x1n = _ln(x1)
  sb = mod(3)
  if GB_AT == 2:
      mcp[5].start()
  cb = mod(4)
  if GB_AT == 3:
      mcp[5].start()
  h3 = _ln(x1n * (1 + cb) + sb)
  hs = [jnp.broadcast_to(h3[:, j * 128:(j + 1) * 128], (CH, 128)) for j in range(D // 128)]

  if MXU:
      w2r = w2_v[...]
      ys = [jnp.zeros((1, 128), f32) for _ in range(D // 128)]
      for i in range(F // CH):
          r = pl.ds(i * CH, CH)
          w1c, b1c = w1b[r, :], b1b[r, :]
          for j in range(D // 128):
              u = w1c * hs[j] + b1c
              g = u * jnp.tanh(u * (u * u + C0 / S3))
              ys[j] = ys[j] + jnp.dot(w2r[:, i * CH:(i + 1) * CH], g.astype(bf16), preferred_element_type=f32)
      y = jnp.concatenate(ys, axis=-1) * (0.5 / S3) + (lin1 * h3 + lin0)
  else:
      accs = [jnp.zeros((8, 128), f32) for _ in range(D // 128)]
      for i in range(F // CH):
          r = pl.ds(i * CH, CH)
          w1c, b1c, w2c = w1b[r, :], b1b[r, :], w2b[r, :]
          for j in range(D // 128):
              u = w1c * hs[j] + b1c
              g = (u * w2c) * jnp.tanh(u * (u * u + C0 / S3))
              accs[j] = accs[j] + g.reshape(CH // 8, 8, 128).sum(axis=0)
      y = jnp.concatenate([jnp.sum(t, axis=0, keepdims=True) for t in accs], axis=-1) + (lin1 * h3 + lin0)
  gb = mod(5)
  o_ref[0] = (x1 + gb * y).astype(o_ref.dtype)

@jax.jit
def pallas_adaLN_cond__sliding_block_cached__mixer_token_mlp__decode_kernel(A_x, A_k_cache, A_v_cache, A_wq, A_wo, B_x, B_w1, B_b1, B_w2, B_b2, c, w_mod):
  kT = jnp.swapaxes(A_k_cache, 2, 3)
  vT = jnp.swapaxes(A_v_cache, 2, 3)
  w2 = B_w2.reshape(1, F)
  return pl.pallas_call(
      _kernel,
      in_specs=[pl.BlockSpec(memory_space=pl.ANY)] * 11,
      out_specs=pl.BlockSpec(memory_space=pltpu.VMEM),
      out_shape=jax.ShapeDtypeStruct((1, 1, D), A_x.dtype),
      scratch_shapes=[
          pltpu.VMEM((NBUF, DH, W), bf16), pltpu.VMEM((NBUF, DH, W), bf16),
          pltpu.VMEM((D, HQ * DH), bf16), pltpu.VMEM((HQ * DH, D), bf16), pltpu.VMEM((6, D, D), bf16),
          pltpu.VMEM((1, 1, D), bf16), pltpu.VMEM((1, F), bf16), pltpu.VMEM((F,), bf16),
          pltpu.VMEM((1, F), bf16), pltpu.VMEM((1,), bf16), pltpu.VMEM((1, D), bf16),
          pltpu.VMEM((HQ, DH), f32),
          pltpu.VMEM((F, 128), f32), pltpu.VMEM((F, 128), f32), pltpu.VMEM((F, 128), f32),
          pltpu.SemaphoreType.DMA((NBUF,)), pltpu.SemaphoreType.DMA((NBUF,)),
          pltpu.SemaphoreType.DMA((2,)), pltpu.SemaphoreType.DMA((6,)), pltpu.SemaphoreType.DMA((6,)),
      ],
      compiler_params=pltpu.CompilerParams(vmem_limit_bytes=100 * 1024 * 1024),
  )(A_x, kT, vT, A_wq, A_wo, B_w1, B_b1, w2, B_b2, c, w_mod)
```

```python
import jax
import jax.numpy as jnp
import numpy as np
from jax import lax
import jax.experimental.pallas as pl
import jax.experimental.pallas.tpu as pltpu

D = 640
HQ = 32
DH = 192
SK = 32768
W = 4096
F = 1536
f32 = jnp.float32
bf16 = jnp.bfloat16
C0 = float(np.sqrt(2.0 / np.pi))
C1 = 0.044715 * C0
S3 = float(C1 ** (1.0 / 3.0))


def _ln(x):
    m = jnp.mean(x, axis=-1, keepdims=True)
    xc = x - m
    v = jnp.mean(xc * xc, axis=-1, keepdims=True)
    return xc / jnp.sqrt(v + 1e-5)


NBUF = 3
CH = 128
EV = (60, 61, 62, 63)


def _kernel(x_hbm, k_hbm, v_hbm, wq_hbm, wo_hbm, w1_hbm, b1_hbm, w2_hbm, b2_hbm, c_hbm, wm_hbm,
          o_ref,
          kbuf, vbuf, wq_v, wo_v, wm_v, x_v, w1_v, b1_v, w2_v, b2_v, c_v, q_s, w1b, b1b,
          ksem, vsem, wsem, msem, ssem):
  def kcopy(h, slot):
      return pltpu.make_async_copy(k_hbm.at[0, h, :, pl.ds(SK - W, W)], kbuf.at[slot], ksem.at[slot])

  def vcopy(h, slot):
      return pltpu.make_async_copy(v_hbm.at[0, h, :, pl.ds(SK - W, W)], vbuf.at[slot], vsem.at[slot])

  small = [pltpu.make_async_copy(s, d, ssem.at[i]) for i, (s, d) in enumerate(
      [(c_hbm, c_v), (x_hbm, x_v), (w1_hbm, w1_v), (b1_hbm, b1_v), (w2_hbm, w2_v), (b2_hbm, b2_v)])]
  mcp = [pltpu.make_async_copy(wm_hbm.at[:, pl.ds(i * D, D)], wm_v.at[i], msem.at[i]) for i in range(6)]
  wq_cp = pltpu.make_async_copy(wq_hbm, wq_v, wsem.at[0])
  wo_cp = pltpu.make_async_copy(wo_hbm, wo_v, wsem.at[1])
  mcp[0].start()
  mcp[1].start()
  for s in small:
      s.start()
  wq_cp.start()
  kcopy(0, 0).start()
  vcopy(0, 0).start()
  wo_cp.start()
  for i in range(1, NBUF):
      kcopy(i, i).start()
      vcopy(i, i).start()
  for s in small:
      s.wait()
  c = c_v[...].astype(f32)
  sc = (c * jax.nn.sigmoid(c)).astype(bf16)
  x = x_v[0].astype(f32)
  xn = _ln(x)
  w1 = w1_v[...].astype(f32)
  b1 = b1_v[...].astype(f32).reshape(1, F)
  hw2 = 0.5 * w2_v[...].astype(f32)
  b2 = b2_v[...].astype(f32).reshape(1, 1)
  w1b[...] = jnp.broadcast_to(w1 * S3, (128, F)).T
  b1b[...] = jnp.broadcast_to(b1 * S3, (128, F)).T
  lin1 = jnp.sum(hw2 * w1, axis=-1, keepdims=True)
  lin0 = jnp.sum(hw2 * b1, axis=-1, keepdims=True) + b2

  def mod(i):
      mcp[i].wait()
      return jnp.dot(sc, wm_v[i], preferred_element_type=f32)

  sa = mod(0)
  ca = mod(1)
  h = xn * (1 + ca) + sa
  wq_cp.wait()
  q = jnp.dot(h.astype(bf16), wq_v[...], preferred_element_type=f32) * (DH ** -0.5)
  for i in range(HQ):
      q_s[i:i + 1, :] = q[:, i * DH:(i + 1) * DH]
  wo_cp.wait()

  def body(hd, acc):
      slot = hd % NBUF
      kcopy(hd, slot).wait()
      qh = q_s[pl.ds(hd, 1), :].astype(bf16)
      s = jnp.dot(qh, kbuf[slot], preferred_element_type=f32)

      @pl.when(hd + NBUF < HQ)
      def _():
          kcopy(hd + NBUF, slot).start()
      def late(stage):
          for j, e in enumerate(EV):
              if e % 2 == stage:
                  pl.when(hd == e // 2)(mcp[2 + j].start)
      late(0)
      m = jnp.max(s, axis=-1, keepdims=True)
      p = jnp.exp(s - m)
      l = jnp.sum(p, axis=-1, keepdims=True)
      vcopy(hd, slot).wait()
      o = lax.dot_general(p.astype(bf16), vbuf[slot], (((1,), (1,)), ((), ())), preferred_element_type=f32)

      @pl.when(hd + NBUF < HQ)
      def _():
          vcopy(hd + NBUF, slot).start()
      late(1)
      o = o / l
      woh = wo_v[pl.ds(pl.multiple_of(hd * DH, DH), DH), :]
      return acc + jnp.dot(o.astype(bf16), woh, preferred_element_type=f32)

  a = lax.fori_loop(0, HQ, body, jnp.zeros((1, D), f32))
  ga = mod(2)
  x1 = x + ga * a
  x1n = _ln(x1)
  sb = mod(3)
  cb = mod(4)
  h3 = _ln(x1n * (1 + cb) + sb)
  hs = [jnp.broadcast_to(h3[:, j * 128:(j + 1) * 128], (CH, 128)) for j in range(D // 128)]

  w2r = w2_v[...]
  ys = [jnp.zeros((1, 128), f32) for _ in range(D // 128)]
  for i in range(F // CH):
      r = pl.ds(i * CH, CH)
      w1c, b1c = w1b[r, :], b1b[r, :]
      for j in range(D // 128):
          u = w1c * hs[j] + b1c
          g = u * jnp.tanh(u * (u * u + C0 / S3))
          ys[j] = ys[j] + jnp.dot(w2r[:, i * CH:(i + 1) * CH], g.astype(bf16), preferred_element_type=f32)
  y = jnp.concatenate(ys, axis=-1) * (0.5 / S3) + (lin1 * h3 + lin0)
  gb = mod(5)
  o_ref[0] = (x1 + gb * y).astype(o_ref.dtype)

@jax.jit
def pallas_adaLN_cond__sliding_block_cached__mixer_token_mlp__decode_kernel(A_x, A_k_cache, A_v_cache, A_wq, A_wo, B_x, B_w1, B_b1, B_w2, B_b2, c, w_mod):
  kT = jnp.swapaxes(A_k_cache, 2, 3)
  vT = jnp.swapaxes(A_v_cache, 2, 3)
  w2 = B_w2.reshape(1, F)
  return pl.pallas_call(
      _kernel,
      in_specs=[pl.BlockSpec(memory_space=pl.ANY)] * 11,
      out_specs=pl.BlockSpec(memory_space=pltpu.VMEM),
      out_shape=jax.ShapeDtypeStruct((1, 1, D), A_x.dtype),
      scratch_shapes=[
          pltpu.VMEM((NBUF, DH, W), bf16), pltpu.VMEM((NBUF, DH, W), bf16),
          pltpu.VMEM((D, HQ * DH), bf16), pltpu.VMEM((HQ * DH, D), bf16), pltpu.VMEM((6, D, D), bf16),
          pltpu.VMEM((1, 1, D), bf16), pltpu.VMEM((1, F), bf16), pltpu.VMEM((F,), bf16),
          pltpu.VMEM((1, F), bf16), pltpu.VMEM((1,), bf16), pltpu.VMEM((1, D), bf16),
          pltpu.VMEM((HQ, DH), f32),
          pltpu.VMEM((F, 128), f32), pltpu.VMEM((F, 128), f32),
          pltpu.SemaphoreType.DMA((NBUF,)), pltpu.SemaphoreType.DMA((NBUF,)),
          pltpu.SemaphoreType.DMA((2,)), pltpu.SemaphoreType.DMA((6,)), pltpu.SemaphoreType.DMA((6,)),
      ],
      compiler_params=pltpu.CompilerParams(vmem_limit_bytes=100 * 1024 * 1024),
  )(A_x, kT, vT, A_wq, A_wo, B_w1, B_b1, w2, B_b2, c, w_mod)
```

```python
import jax
import jax.numpy as jnp
import numpy as np
from jax import lax
import jax.experimental.pallas as pl
import jax.experimental.pallas.tpu as pltpu

D = 640
HQ = 32
DH = 192
SK = 32768
W = 4096
F = 1536
f32 = jnp.float32
bf16 = jnp.bfloat16
C0 = float(np.sqrt(2.0 / np.pi))
C1 = 0.044715 * C0
S3 = float(C1 ** (1.0 / 3.0))


def _ln(x):
    m = jnp.mean(x, axis=-1, keepdims=True)
    xc = x - m
    v = jnp.mean(xc * xc, axis=-1, keepdims=True)
    return xc / jnp.sqrt(v + 1e-5)


NBUF = 3
CH = 128
EV = (60, 61, 62, 63)


def _kernel(x_hbm, k_hbm, v_hbm, wq_hbm, wo_hbm, w1_hbm, b1_hbm, w2_hbm, b2_hbm, c_hbm, wm_hbm,
          o_ref,
          kbuf, vbuf, wq_v, wo_v, wm_v, x_v, w1_v, b1_v, w2_v, b2_v, c_v, q_s, w1b, b1b,
          ksem, vsem, wsem, msem, ssem):
  def kcopy(h, slot):
      return pltpu.make_async_copy(k_hbm.at[0, h, :, pl.ds(SK - W, W)], kbuf.at[slot], ksem.at[slot])

  def vcopy(h, slot):
      return pltpu.make_async_copy(v_hbm.at[0, h, :, pl.ds(SK - W, W)], vbuf.at[slot], vsem.at[slot])

  small = [pltpu.make_async_copy(s, d, ssem.at[i]) for i, (s, d) in enumerate(
      [(c_hbm, c_v), (x_hbm, x_v), (w1_hbm, w1_v), (b1_hbm, b1_v), (w2_hbm, w2_v), (b2_hbm, b2_v)])]
  mcp = [pltpu.make_async_copy(wm_hbm.at[:, pl.ds(i * D, D)], wm_v.at[i], msem.at[i]) for i in range(6)]
  wq_cp = pltpu.make_async_copy(wq_hbm, wq_v, wsem.at[0])
  wo_cp = pltpu.make_async_copy(wo_hbm, wo_v, wsem.at[1])
  mcp[0].start()
  mcp[1].start()
  for s in small:
      s.start()
  wq_cp.start()
  kcopy(0, 0).start()
  vcopy(0, 0).start()
  wo_cp.start()
  for i in range(1, NBUF):
      kcopy(i, i).start()
      vcopy(i, i).start()
  for s in small:
      s.wait()
  c = c_v[...].astype(f32)
  sc = (c * jax.nn.sigmoid(c)).astype(bf16)
  x = x_v[0].astype(f32)
  xn = _ln(x)
  w1 = w1_v[...].astype(f32)
  b1 = b1_v[...].astype(f32).reshape(1, F)
  hw2 = 0.5 * w2_v[...].astype(f32)
  b2 = b2_v[...].astype(f32).reshape(1, 1)
  w1b[...] = jnp.broadcast_to(w1 * S3, (128, F)).T
  b1b[...] = jnp.broadcast_to(b1 * S3, (128, F)).T
  lin1 = jnp.sum(hw2 * w1, axis=-1, keepdims=True)
  lin0 = jnp.sum(hw2 * b1, axis=-1, keepdims=True) + b2

  p1 = hw2 * w1
  p0 = hw2 * b1
  p1h = p1.astype(bf16).astype(f32)
  p0h = p0.astype(bf16).astype(f32)
  coef = jnp.concatenate([p1h, p1 - p1h, p0h, p0 - p0h, jnp.zeros((12, F), f32)], axis=0).astype(bf16)

  def mod(i):
      mcp[i].wait()
      return jnp.dot(sc, wm_v[i], preferred_element_type=f32)

  sa = mod(0)
  ca = mod(1)
  h = xn * (1 + ca) + sa
  wq_cp.wait()
  q = jnp.dot(h.astype(bf16), wq_v[...], preferred_element_type=f32) * (DH ** -0.5)
  for i in range(HQ):
      q_s[i:i + 1, :] = q[:, i * DH:(i + 1) * DH]
  wo_cp.wait()

  def body(hd, acc):
      slot = hd % NBUF
      kcopy(hd, slot).wait()
      qh = q_s[pl.ds(hd, 1), :].astype(bf16)
      s = jnp.dot(qh, kbuf[slot], preferred_element_type=f32)

      @pl.when(hd + NBUF < HQ)
      def _():
          kcopy(hd + NBUF, slot).start()
      def late(stage):
          for j, e in enumerate(EV):
              if e % 2 == stage:
                  pl.when(hd == e // 2)(mcp[2 + j].start)
      late(0)
      m = jnp.max(s, axis=-1, keepdims=True)
      p = jnp.exp(s - m)
      l = jnp.sum(p, axis=-1, keepdims=True)
      vcopy(hd, slot).wait()
      o = lax.dot_general(p.astype(bf16), vbuf[slot], (((1,), (1,)), ((), ())), preferred_element_type=f32)

      @pl.when(hd + NBUF < HQ)
      def _():
          vcopy(hd + NBUF, slot).start()
      late(1)
      o = o / l
      woh = wo_v[pl.ds(pl.multiple_of(hd * DH, DH), DH), :]
      return acc + jnp.dot(o.astype(bf16), woh, preferred_element_type=f32)

  a = lax.fori_loop(0, HQ, body, jnp.zeros((1, D), f32))
  ga = mod(2)
  x1 = x + ga * a
  x1n = _ln(x1)
  sb = mod(3)
  cb = mod(4)
  h3 = _ln(x1n * (1 + cb) + sb)
  hs = [jnp.broadcast_to(h3[:, j * 128:(j + 1) * 128], (CH, 128)) for j in range(D // 128)]

  ys = [jnp.zeros((16, 128), f32) for _ in range(D // 128)]
  for i in range(F // CH):
      r = pl.ds(i * CH, CH)
      w1c, b1c = w1b[r, :], b1b[r, :]
      for j in range(D // 128):
          u = w1c * hs[j] + b1c
          t = jnp.tanh(u * (u * u + C0 / S3))
          ys[j] = ys[j] + jnp.dot(coef[:, i * CH:(i + 1) * CH], t.astype(bf16), preferred_element_type=f32)
  yy = jnp.concatenate(ys, axis=-1)
  y = (yy[0:1] + yy[1:2] + lin1) * h3 + (yy[2:3] + yy[3:4] + lin0)
  gb = mod(5)
  o_ref[0] = (x1 + gb * y).astype(o_ref.dtype)

@jax.jit
def pallas_adaLN_cond__sliding_block_cached__mixer_token_mlp__decode_kernel(A_x, A_k_cache, A_v_cache, A_wq, A_wo, B_x, B_w1, B_b1, B_w2, B_b2, c, w_mod):
  kT = jnp.swapaxes(A_k_cache, 2, 3)
  vT = jnp.swapaxes(A_v_cache, 2, 3)
  w2 = B_w2.reshape(1, F)
  return pl.pallas_call(
      _kernel,
      in_specs=[pl.BlockSpec(memory_space=pl.ANY)] * 11,
      out_specs=pl.BlockSpec(memory_space=pltpu.VMEM),
      out_shape=jax.ShapeDtypeStruct((1, 1, D), A_x.dtype),
      scratch_shapes=[
          pltpu.VMEM((NBUF, DH, W), bf16), pltpu.VMEM((NBUF, DH, W), bf16),
          pltpu.VMEM((D, HQ * DH), bf16), pltpu.VMEM((HQ * DH, D), bf16), pltpu.VMEM((6, D, D), bf16),
          pltpu.VMEM((1, 1, D), bf16), pltpu.VMEM((1, F), bf16), pltpu.VMEM((F,), bf16),
          pltpu.VMEM((1, F), bf16), pltpu.VMEM((1,), bf16), pltpu.VMEM((1, D), bf16),
          pltpu.VMEM((HQ, DH), f32),
          pltpu.VMEM((F, 128), f32), pltpu.VMEM((F, 128), f32),
          pltpu.SemaphoreType.DMA((NBUF,)), pltpu.SemaphoreType.DMA((NBUF,)),
          pltpu.SemaphoreType.DMA((2,)), pltpu.SemaphoreType.DMA((6,)), pltpu.SemaphoreType.DMA((6,)),
      ],
      compiler_params=pltpu.CompilerParams(vmem_limit_bytes=100 * 1024 * 1024),
  )(A_x, kT, vT, A_wq, A_wo, B_w1, B_b1, w2, B_b2, c, w_mod)
```

```python
import jax
import jax.numpy as jnp
import numpy as np
from jax import lax
import jax.experimental.pallas as pl
import jax.experimental.pallas.tpu as pltpu

D = 640
HQ = 32
DH = 192
SK = 32768
W = 4096
F = 1536
f32 = jnp.float32
bf16 = jnp.bfloat16
C0 = float(np.sqrt(2.0 / np.pi))
C1 = 0.044715 * C0
S3 = float(C1 ** (1.0 / 3.0))


def _ln(x):
    m = jnp.mean(x, axis=-1, keepdims=True)
    xc = x - m
    v = jnp.mean(xc * xc, axis=-1, keepdims=True)
    return xc / jnp.sqrt(v + 1e-5)


NBUF = 3
CH = 128
GBI = 10
SPLIT = 5
EV = (60, 61, 62, 63)


def _kernel(x_hbm, k_hbm, v_hbm, wq_hbm, wo_hbm, w1_hbm, b1_hbm, w2_hbm, b2_hbm, c_hbm, wm_hbm,
          o_ref,
          kbuf, vbuf, wq_v, wo_v, wm_v, x_v, w1_v, b1_v, w2_v, b2_v, c_v, q_s, w1b, b1b,
          ksem, vsem, wsem, msem, ssem, csem):
  def kcopy(h, slot):
      return pltpu.make_async_copy(k_hbm.at[0, h, :, pl.ds(SK - W, W)], kbuf.at[slot], ksem.at[slot])

  def vcopy(h, slot):
      return pltpu.make_async_copy(v_hbm.at[0, h, :, pl.ds(SK - W, W)], vbuf.at[slot], vsem.at[slot])

  small = [pltpu.make_async_copy(s, d, ssem.at[i]) for i, (s, d) in enumerate(
      [(c_hbm, c_v), (x_hbm, x_v), (w1_hbm, w1_v), (b1_hbm, b1_v), (w2_hbm, w2_v), (b2_hbm, b2_v)])]
  mcp = {i: pltpu.make_async_copy(wm_hbm.at[:, pl.ds(i * D, D)], wm_v.at[i], msem.at[i]) for i in (0, 1, 2, 3, 5)}
  RS = D // SPLIT
  ccp = [pltpu.make_async_copy(wm_hbm.at[pl.ds(r * RS, RS), pl.ds(4 * D, D)], wm_v.at[4, pl.ds(r * RS, RS)], csem.at[r]) for r in range(SPLIT)]

  def start_mod(i):
      if i == 4:
          for cc in ccp:
              cc.start()
      else:
          mcp[i].start()
  wq_cp = pltpu.make_async_copy(wq_hbm, wq_v, wsem.at[0])
  wo_cp = pltpu.make_async_copy(wo_hbm, wo_v, wsem.at[1])
  mcp[0].start()
  mcp[1].start()
  for s in small:
      s.start()
  wq_cp.start()
  kcopy(0, 0).start()
  vcopy(0, 0).start()
  wo_cp.start()
  for i in range(1, NBUF):
      kcopy(i, i).start()
      vcopy(i, i).start()
  for s in small:
      s.wait()
  c = c_v[...].astype(f32)
  sc = (c * jax.nn.sigmoid(c)).astype(bf16)
  x = x_v[0].astype(f32)
  xn = _ln(x)
  w1 = w1_v[...].astype(f32)
  b1 = b1_v[...].astype(f32).reshape(1, F)
  hw2 = 0.5 * w2_v[...].astype(f32)
  b2 = b2_v[...].astype(f32).reshape(1, 1)
  w1b[...] = jnp.broadcast_to(w1 * S3, (128, F)).T
  b1b[...] = jnp.broadcast_to(b1 * S3, (128, F)).T
  lin1 = jnp.sum(hw2 * w1, axis=-1, keepdims=True)
  lin0 = jnp.sum(hw2 * b1, axis=-1, keepdims=True) + b2

  p1 = hw2 * w1
  p0 = hw2 * b1
  p1h = p1.astype(bf16).astype(f32)
  p0h = p0.astype(bf16).astype(f32)
  coef = jnp.concatenate([p1h, p1 - p1h, p0h, p0 - p0h, jnp.zeros((12, F), f32)], axis=0).astype(bf16)

  def mod(i):
      mcp[i].wait()
      return jnp.dot(sc, wm_v[i], preferred_element_type=f32)

  sa = mod(0)
  ca = mod(1)
  h = xn * (1 + ca) + sa
  wq_cp.wait()
  q = jnp.dot(h.astype(bf16), wq_v[...], preferred_element_type=f32) * (DH ** -0.5)
  for i in range(HQ):
      q_s[i:i + 1, :] = q[:, i * DH:(i + 1) * DH]
  wo_cp.wait()

  def body(hd, acc):
      slot = hd % NBUF
      kcopy(hd, slot).wait()
      qh = q_s[pl.ds(hd, 1), :].astype(bf16)
      s = jnp.dot(qh, kbuf[slot], preferred_element_type=f32)

      @pl.when(hd + NBUF < HQ)
      def _():
          kcopy(hd + NBUF, slot).start()
      def late(stage):
          for j, e in enumerate(EV):
              if e % 2 == stage:
                  pl.when(hd == e // 2)(lambda j=j: start_mod(2 + j))
      late(0)
      m = jnp.max(s, axis=-1, keepdims=True)
      p = jnp.exp(s - m)
      l = jnp.sum(p, axis=-1, keepdims=True)
      vcopy(hd, slot).wait()
      o = lax.dot_general(p.astype(bf16), vbuf[slot], (((1,), (1,)), ((), ())), preferred_element_type=f32)

      @pl.when(hd + NBUF < HQ)
      def _():
          vcopy(hd + NBUF, slot).start()
      late(1)
      o = o / l
      woh = wo_v[pl.ds(pl.multiple_of(hd * DH, DH), DH), :]
      return acc + jnp.dot(o.astype(bf16), woh, preferred_element_type=f32)

  a = lax.fori_loop(0, HQ, body, jnp.zeros((1, D), f32))
  ga = mod(2)
  x1 = x + ga * a
  x1n = _ln(x1)
  sb = mod(3)
  cb = jnp.zeros((1, D), f32)
  for r in range(SPLIT):
      ccp[r].wait()
      cb = cb + jnp.dot(sc[:, r * RS:(r + 1) * RS], wm_v[4, r * RS:(r + 1) * RS, :], preferred_element_type=f32)
  h3 = _ln(x1n * (1 + cb) + sb)
  hs = [jnp.broadcast_to(h3[:, j * 128:(j + 1) * 128], (CH, 128)) for j in range(D // 128)]

  ys = [jnp.zeros((16, 128), f32) for _ in range(D // 128)]
  for i in range(F // CH):
      r = pl.ds(i * CH, CH)
      w1c, b1c = w1b[r, :], b1b[r, :]
      if i == GBI:
          gb = mod(5)
      for j in range(D // 128):
          u = w1c * hs[j] + b1c
          t = jnp.tanh(u * (u * u + C0 / S3))
          ys[j] = ys[j] + jnp.dot(coef[:, i * CH:(i + 1) * CH], t.astype(bf16), preferred_element_type=f32)
  yy = jnp.concatenate(ys, axis=-1)
  y = (yy[0:1] + yy[1:2] + lin1) * h3 + (yy[2:3] + yy[3:4] + lin0)
  o_ref[0] = (x1 + gb * y).astype(o_ref.dtype)

@jax.jit
def pallas_adaLN_cond__sliding_block_cached__mixer_token_mlp__decode_kernel(A_x, A_k_cache, A_v_cache, A_wq, A_wo, B_x, B_w1, B_b1, B_w2, B_b2, c, w_mod):
  kT = jnp.swapaxes(A_k_cache, 2, 3)
  vT = jnp.swapaxes(A_v_cache, 2, 3)
  w2 = B_w2.reshape(1, F)
  return pl.pallas_call(
      _kernel,
      in_specs=[pl.BlockSpec(memory_space=pl.ANY)] * 11,
      out_specs=pl.BlockSpec(memory_space=pltpu.VMEM),
      out_shape=jax.ShapeDtypeStruct((1, 1, D), A_x.dtype),
      scratch_shapes=[
          pltpu.VMEM((NBUF, DH, W), bf16), pltpu.VMEM((NBUF, DH, W), bf16),
          pltpu.VMEM((D, HQ * DH), bf16), pltpu.VMEM((HQ * DH, D), bf16), pltpu.VMEM((6, D, D), bf16),
          pltpu.VMEM((1, 1, D), bf16), pltpu.VMEM((1, F), bf16), pltpu.VMEM((F,), bf16),
          pltpu.VMEM((1, F), bf16), pltpu.VMEM((1,), bf16), pltpu.VMEM((1, D), bf16),
          pltpu.VMEM((HQ, DH), f32),
          pltpu.VMEM((F, 128), f32), pltpu.VMEM((F, 128), f32),
          pltpu.SemaphoreType.DMA((NBUF,)), pltpu.SemaphoreType.DMA((NBUF,)),
          pltpu.SemaphoreType.DMA((2,)), pltpu.SemaphoreType.DMA((6,)), pltpu.SemaphoreType.DMA((6,)),
          pltpu.SemaphoreType.DMA((SPLIT,)),
      ],
      compiler_params=pltpu.CompilerParams(vmem_limit_bytes=100 * 1024 * 1024),
  )(A_x, kT, vT, A_wq, A_wo, B_w1, B_b1, w2, B_b2, c, w_mod)
```
